```python
import jax
import jax.numpy as jnp

def _softmax(x, axis=-1):
    return jax.nn.softmax(x, axis=axis)
def _gelu(x):
    return jax.nn.gelu(x, approximate=True)
def _silu(x):
    return jax.nn.silu(x)
def _sigmoid(x):
    return jax.nn.sigmoid(x)
def _layernorm(x, axis=-1, eps=1e-5):
    m = jnp.mean(x, axis=axis, keepdims=True)
    v = jnp.var(x, axis=axis, keepdims=True)
    return (x - m) / jnp.sqrt(v + eps)
def _scatter_add(tgt, idx, src, axis=0):
    return tgt.at[idx].add(src)
def _segment_sum(src, seg, n):
    return jax.ops.segment_sum(src, seg, n)
class _Rng:
    def __init__(self, key):
        self._k = key
    def _next(self):
        self._k, sub = jax.random.split(self._k)
        return sub
    def normal(self, shape):
        return jax.random.normal(self._next(), shape, dtype=jnp.bfloat16)
    def randint(self, lo, hi, shape):
        return jax.random.randint(self._next(), shape, lo, hi, dtype=jnp.int32)
    def uniform(self, shape, lo=0.0, hi=1.0):
        return jax.random.uniform(self._next(), shape, jnp.bfloat16, lo, hi)
    def permutation(self, n):
        return jax.random.permutation(self._next(), n)


kernel_name = 'interleave_layers__sliding_block_cached__dense_activation_gelu__decode'

def _fwd_setup_inputs():
    _rng = _Rng(jax.random.key(int.from_bytes(__import__("os").urandom(4), "little")))
    _w = (lambda a: (lambda t: t.astype(jnp.bfloat16) if jnp.issubdtype(t.dtype, jnp.floating) else t)(jnp.asarray(a)))
    def _A_setup():
        B, Sq, D = 2, 1, 512
        Hq, Hkv, Sk, Dh = 32, 8, 32768, 128
        assert Hq % Hkv == 0, (Hq, Hkv)
        return {
            "x": _w((lambda *s: _rng.normal(s) * 0.05)(B, Sq, D)),
            "k_cache": _w((lambda *s: _rng.normal(s) * 0.05)(B, Hkv, Sk, Dh)),
            "v_cache": _w((lambda *s: _rng.normal(s) * 0.05)(B, Hkv, Sk, Dh)),
            "wq": _w((lambda *s: _rng.normal(s) * 0.05)(D, Hq * Dh) * (D ** -0.5)),
            "wo": _w((lambda *s: _rng.normal(s) * 0.05)(Hq * Dh, D) * ((Hq * Dh) ** -0.5)),
        }
    _A_in = _A_setup()

    def _B_setup():
        B, S, D, F = 2, 1, 512, 1792
        return {
            "x": _w((lambda *s: _rng.normal(s) * 0.05)(B, S, D)),
            "w1": _w((lambda *s: _rng.normal(s) * 0.05)(D, F) * (D ** -0.5)),
            "b1": _w((lambda *s: _rng.normal(s) * 0.05)(F) * 0.01),
            "w2": _w((lambda *s: _rng.normal(s) * 0.05)(F, D) * (F ** -0.5)),
            "b2": _w((lambda *s: _rng.normal(s) * 0.05)(D) * 0.01),
        }
    _B_in = _B_setup()

    return {
        "A_x": _A_in["x"],
        "A_k_cache": _A_in["k_cache"],
        "A_v_cache": _A_in["v_cache"],
        "A_wq": _A_in["wq"],
        "A_wo": _A_in["wo"],
        "B_x": _B_in["x"],
        "B_w1": _B_in["w1"],
        "B_b1": _B_in["b1"],
        "B_w2": _B_in["w2"],
        "B_b2": _B_in["b2"],
    }

def _fwd_reference(A_x, A_k_cache, A_v_cache, A_wq, A_wo, B_x, B_w1, B_b1, B_w2, B_b2):
    def _A_ref(x, k_cache, v_cache, wq, wo):
        B, Sq, D = x.shape
        Hq, Dh = 32, 128
        Hkv, Sk = k_cache.shape[1], k_cache.shape[2]
        W = min(4096, max(256, Sk // 4))
        rep = Hq // Hkv
        q = (lambda x, *d: x.transpose(*d))((x @ wq).reshape(B, Sq, Hq, Dh), 0, 2, 1, 3)
        k = jnp.repeat(k_cache[:, :, Sk - W:, :], rep, axis=1)
        v = jnp.repeat(v_cache[:, :, Sk - W:, :], rep, axis=1)
        scores = jnp.einsum("bhqd,bhkd->bhqk", q, k) * (Dh ** -0.5)
        p = _softmax(scores, axis=-1)
        o = jnp.einsum("bhqk,bhkd->bhqd", p, v)
        return (lambda x, *d: x.transpose(*d))(o, 0, 2, 1, 3).reshape(B, Sq, Hq * Dh) @ wo

    def _B_ref(x, w1, b1, w2, b2):
        h = jnp.einsum("bsd,df->bsf", x, w1) + b1
        h = _gelu(h)
        return jnp.einsum("bsf,fd->bsd", h, w2) + b2

    x = A_x
    x = x + _A_ref(_layernorm(x, axis=-1), A_k_cache, A_v_cache, A_wq, A_wo)
    x = x + _B_ref(_layernorm(x, axis=-1), B_w1, B_b1, B_w2, B_b2)
    x = x + _A_ref(_layernorm(x, axis=-1), A_k_cache, A_v_cache, A_wq, A_wo)
    x = x + _B_ref(_layernorm(x, axis=-1), B_w1, B_b1, B_w2, B_b2)
    return x


def setup_inputs():
    _inp = _fwd_setup_inputs()
    _gk = jax.random.fold_in(jax.random.key(int.from_bytes(__import__("os").urandom(4), "little")), 2**31 - 1)
    _shapes = [[2, 1, 512]]
    _dtypes = ['bfloat16']
    _gks = jax.random.split(_gk, len(_shapes))
    _gs = [jax.random.normal(k, s, dtype=jnp.dtype(d)) * 0.05 for k, s, d in zip(_gks, _shapes, _dtypes)]
    _inp["grad_out"] = _gs[0]
    return _inp

def reference(A_x, A_k_cache, A_v_cache, A_wq, A_wo, B_w1, B_b1, B_w2, B_b2, B_x, grad_out):
    _const = dict(B_x=B_x)
    def _f(*_d):
        return _fwd_reference(**{'A_x': _d[0], 'A_k_cache': _d[1], 'A_v_cache': _d[2], 'A_wq': _d[3], 'A_wo': _d[4], 'B_w1': _d[5], 'B_b1': _d[6], 'B_w2': _d[7], 'B_b2': _d[8], **_const})
    _out, _vjp = jax.vjp(_f, A_x, A_k_cache, A_v_cache, A_wq, A_wo, B_w1, B_b1, B_w2, B_b2)
    _grads = _vjp(grad_out)
    _out0 = jnp.asarray(_out)
    return (_out0, *[jnp.asarray(_g) for _g in _grads])
```

```python
import math

import jax
import jax.numpy as jnp
from jax import lax
import jax.experimental.pallas as pl
import jax.experimental.pallas.tpu as pltpu

_F32 = jnp.float32
_BF16 = jnp.bfloat16
_EPS = 1e-5
_GELU_C = math.sqrt(2.0 / math.pi)
_GELU_A = 0.044715
_PIECE = 128


def _mm(a, b):
  return lax.dot_general(a.astype(_BF16), b, (((1,), (0,)), ((), ())),
                         preferred_element_type=_F32)


def _mm_nt(a, b):
  return lax.dot_general(a.astype(_BF16), b, (((1,), (1,)), ((), ())),
                         preferred_element_type=_F32)


def _mm_tn(a, b):
  return lax.dot_general(a.astype(_BF16), b.astype(_BF16),
                         (((0,), (0,)), ((), ())), preferred_element_type=_F32)


def _rows(n):
  return lax.broadcasted_iota(jnp.int32, (8, n), 0)


def _ln_fwd(x):
  xc = x - jnp.mean(x, axis=-1, keepdims=True)
  var = jnp.mean(xc * xc, axis=-1, keepdims=True)
  rstd = 1.0 / jnp.sqrt(var + _EPS)
  return xc * rstd, rstd


def _ln_bwd(dn, n, rstd):
  return rstd * (dn - jnp.mean(dn, axis=-1, keepdims=True)
                 - n * jnp.mean(dn * n, axis=-1, keepdims=True))


def _gelu(h):
  t = jnp.tanh(_GELU_C * (h + _GELU_A * h * h * h))
  g = 0.5 * h * (1.0 + t)
  dg = 0.5 * (1.0 + t) + 0.5 * h * (1.0 - t * t) * _GELU_C * (
      1.0 + 3.0 * _GELU_A * h * h)
  return g, dg


def _sum_over_r(a):
  a = a + pltpu.roll(a, 4, 0)
  return a + pltpu.roll(a, 2, 0)


def _make_kernel(nb, hkv, rep, dh, seq, win, d, f, zero_plan):
  w0 = seq - win
  nzero = nb * (w0 // _PIECE)
  scale = dh ** -0.5
  hd = hkv * rep * dh

  def kernel(x_h, go_h, k_h, v_h, wq_h, wo_h, w1_h, b1_h, w2_h, b2_h,
             out_h, dx_h, dk_h, dv_h, dwq_h, dwo_h, dw1_h, db1_h, dw2_h, db2_h,
             x_s, go_s, k_s, v_s, wq_s, wo_s, w1_s, b1_s, w2_s, b2_s,
             out_s, dx_s, dk_s, dv_s, dwq_s, dwo_s, dw1_s, db1_s, dw2_s, db2_s,
             z_s, q_s, o_s, do_s, dq_s, p_s, ds_s,
             rsem, ksem, vsem, zsem, wsem):

    small_in = [
        pltpu.make_async_copy(src, dst, rsem.at[i]) for i, (src, dst) in
        enumerate(((x_h, x_s), (go_h, go_s), (b1_h, b1_s), (b2_h, b2_s)))]
    wq_in = pltpu.make_async_copy(wq_h, wq_s, rsem.at[4])
    wo_in = pltpu.make_async_copy(wo_h, wo_s, rsem.at[5])
    w1_in = pltpu.make_async_copy(w1_h, w1_s, rsem.at[6])
    w2_in = pltpu.make_async_copy(w2_h, w2_s, rsem.at[7])

    def k_in(h):
      return pltpu.make_async_copy(
          k_h.at[:, h, pl.ds(w0, win)], k_s.at[h], ksem.at[h])

    def v_in(h):
      return pltpu.make_async_copy(
          v_h.at[:, h, pl.ds(w0, win)], v_s.at[h], vsem.at[h])

    wq_in.start()
    for c in small_in:
      c.start()
    for h in range(hkv):
      k_in(h).start()
      v_in(h).start()
    wo_in.start()
    w1_in.start()
    w2_in.start()

    z_s[...] = jnp.zeros(z_s.shape, z_s.dtype)

    def zero_out(dst_h, i):
      per_b = w0 // _PIECE
      row = pl.multiple_of((i % per_b) * _PIECE, _PIECE)
      return pltpu.make_async_copy(
          z_s, dst_h.at[i // per_b, :, pl.ds(row, _PIECE)], zsem.at[0])

    issued = [0]

    def zero_run(n):
      while n > 0:
        which, lo = divmod(issued[0], nzero)
        m = min(n, nzero - lo)
        dst_h = (dk_h, dv_h)[which]

        def body(i, carry, dst_h=dst_h):
          zero_out(dst_h, i).start()
          return carry

        lax.fori_loop(lo, lo + m, body, 0)
        issued[0] += m
        n -= m

    def zero_in_loop(n):
      which, lo = divmod(issued[0], nzero)
      assert lo + n * hkv <= nzero
      dst_h = (dk_h, dv_h)[which]
      issued[0] += n * hkv

      def issue(h):
        def body(i, carry):
          zero_out(dst_h, lo + h * n + i).start()
          return carry

        lax.fori_loop(0, n, body, 0)

      return issue

    odd_d = _rows(d) % 2 == 1
    odd_h = _rows(dh) % 2 == 1
    odd_w = _rows(win) % 2 == 1
    r_h = _rows(dh) // 2

    def load_pair(ref):
      return jnp.where(odd_d,
                       jnp.broadcast_to(ref[1:2].astype(_F32), (8, d)),
                       jnp.broadcast_to(ref[0:1].astype(_F32), (8, d)))

    def to_heads(big, dst, layer):
      for h in range(hkv):
        t = big[:, h * rep * dh:(h * rep + 1) * dh]
        for r in range(1, rep):
          j = h * rep + r
          t = jnp.where(r_h == r, big[:, j * dh:(j + 1) * dh], t)
        dst[h, layer * 8:(layer + 1) * 8, :] = t

    def from_heads(src, layer):
      tiles = []
      for h in range(hkv):
        t = src[h, layer * 8:(layer + 1) * 8, :]
        for r in range(rep):
          tiles.append(jnp.where(r_h == r, t, 0.0))
      return jnp.concatenate(tiles, axis=1)

    def attn_fwd(x, layer, per_head):
      n, rstd = _ln_fwd(x)
      to_heads(_mm(n, wq_s[...]), q_s, layer)
      rows = slice(layer * 8, (layer + 1) * 8)

      def head(h, carry):
        per_head(h)
        q = q_s[h, rows, :]
        s = jnp.where(odd_w, _mm_nt(q, k_s[h, 1]), _mm_nt(q, k_s[h, 0])) * scale
        e = jnp.exp(s - jnp.max(s, axis=-1, keepdims=True))
        p = e / jnp.sum(e, axis=-1, keepdims=True)
        p_s[h, rows, :] = p
        o_s[h, rows, :] = jnp.where(odd_h, _mm(p, v_s[h, 1]), _mm(p, v_s[h, 0]))
        return carry

      lax.fori_loop(0, hkv, head, 0)
      return n, rstd

    def attn_out(layer):
      return _sum_over_r(_mm(from_heads(o_s, layer), wo_s[...]))

    def attn_bwd(da, layer, per_head):
      to_heads(_mm_nt(da, wo_s[...]), do_s, layer)
      rows = slice(layer * 8, (layer + 1) * 8)

      def head(h, carry):
        per_head(h)
        do = do_s[h, rows, :]
        p = p_s[h, rows, :]
        dp = jnp.where(odd_w, _mm_nt(do, v_s[h, 1]), _mm_nt(do, v_s[h, 0]))
        ds = p * (dp - jnp.sum(p * dp, axis=-1, keepdims=True)) * scale
        ds_s[h, rows, :] = ds
        dq_s[h, rows, :] = jnp.where(
            odd_h, _mm(ds, k_s[h, 1]), _mm(ds, k_s[h, 0]))
        return carry

      lax.fori_loop(0, hkv, head, 0)
      return _sum_over_r(_mm_nt(from_heads(dq_s, layer), wq_s[...]))

    def mlp_fwd(x):
      n, rstd = _ln_fwd(x)
      g, dg = _gelu(_mm(n, w1_s[...]) + b1)
      return x + _mm(g, w2_s[...]) + b2, (n, rstd, g, dg)

    def mlp_bwd(dy, saved):
      n, rstd, _, dg = saved
      dh_ = _mm_nt(dy, w2_s[...]) * dg
      return dy + _ln_bwd(_mm_nt(dh_, w1_s[...]), n, rstd), dh_

    for c in small_in:
      c.wait()
    x0 = load_pair(x_s)
    g4 = load_pair(go_s)
    b1 = b1_s[...].astype(_F32).reshape(1, f)
    b2 = b2_s[...].astype(_F32).reshape(1, d)
    wq_in.wait()

    def wait_kv(h):
      k_in(h).wait()
      v_in(h).wait()

    n1, rstd1 = attn_fwd(x0, 0, wait_kv)
    wo_in.wait()
    x1 = x0 + attn_out(0)
    w1_in.wait()
    zero_run(zero_plan[0])
    w2_in.wait()
    x2, mlp2 = mlp_fwd(x1)
    n3, rstd3 = attn_fwd(x2, 1, zero_in_loop(zero_plan[1]))
    x3 = x2 + attn_out(1)
    x4, mlp4 = mlp_fwd(x3)
    out_s[...] = x4[0:nb].astype(out_s.dtype)

    zero_run(zero_plan[2])
    g3, dh4 = mlp_bwd(g4, mlp4)
    g2 = g3 + _ln_bwd(attn_bwd(g3, 1, zero_in_loop(zero_plan[3])), n3, rstd3)
    zero_run(zero_plan[4])
    g1, dh2 = mlp_bwd(g2, mlp2)
    g0 = g1 + _ln_bwd(attn_bwd(g1, 0, zero_in_loop(zero_plan[5])), n1, rstd1)
    dx_s[...] = g0[0:nb].astype(dx_s.dtype)

    zero_run(zero_plan[6])

    def one_r(a):
      return jnp.where(_rows(a.shape[1]) < nb, a, 0.0)

    dm = jnp.concatenate([one_r(g2), one_r(g4)], axis=0)
    dhh = jnp.concatenate([one_r(dh2), one_r(dh4)], axis=0)
    db2_s[...] = jnp.sum(dm, axis=0, keepdims=True).reshape(d).astype(db2_s.dtype)
    db1_s[...] = jnp.sum(dhh, axis=0, keepdims=True).reshape(f).astype(db1_s.dtype)

    def outer(a, b, dst, chunk):
      b = b.astype(_BF16)
      for i in range(0, a.shape[1], chunk):
        dst[i:i + chunk, :] = _mm_tn(a[:, i:i + chunk], b).astype(dst.dtype)

    outer(jnp.concatenate([mlp2[0], mlp4[0]], axis=0), dhh, dw1_s, 128)
    outer(jnp.concatenate([mlp2[2], mlp4[2]], axis=0), dm, dw2_s, 256)
    zero_run(zero_plan[7])
    outer(jnp.concatenate([n1, n3], axis=0),
          jnp.concatenate([from_heads(dq_s, 0), from_heads(dq_s, 1)], axis=0),
          dwq_s, 128)
    zero_run(zero_plan[8])
    outer(jnp.concatenate([from_heads(o_s, 0), from_heads(o_s, 1)], axis=0),
          jnp.concatenate([g1, g3], axis=0), dwo_s, 512)

    grads_out = [
        pltpu.make_async_copy(src, dst, wsem.at[0]) for src, dst in (
            (out_s, out_h), (dx_s, dx_h), (dwq_s, dwq_h), (dwo_s, dwo_h),
            (dw1_s, dw1_h), (db1_s, db1_h), (dw2_s, dw2_h), (db2_s, db2_h))]
    for c in grads_out:
      c.start()

    odd_h16 = lax.broadcasted_iota(jnp.int32, (16, dh), 0) % 2 == 1
    per_head = zero_in_loop(zero_plan[9])
    chunk = 512

    def head(h, carry):
      per_head(h)
      for lhs_s, rhs_s, dst in ((ds_s, q_s, dk_s), (p_s, do_s, dv_s)):
        t = rhs_s[h]
        rhs = jnp.concatenate(
            [jnp.where(odd_h16, 0.0, t), jnp.where(odd_h16, t, 0.0)],
            axis=1).astype(_BF16)
        for i in range(0, win, chunk):
          r = _mm_tn(lhs_s[h, :, i:i + chunk], rhs).astype(dst.dtype)
          dst[h, 0, i:i + chunk, :] = r[:, :dh]
          dst[h, 1, i:i + chunk, :] = r[:, dh:]
      return carry

    lax.fori_loop(0, hkv, head, 0)

    npiece = win // _PIECE

    def win_out(src, dst_h, i):
      row = pl.multiple_of((i % npiece) * _PIECE, _PIECE)
      return pltpu.make_async_copy(
          src.at[:, i // npiece, pl.ds(row, _PIECE)],
          dst_h.at[i // npiece, :, pl.ds(w0 + row, _PIECE)], wsem.at[0])

    def for_each(n, fn):
      def body(i, carry):
        fn(i)
        return carry

      lax.fori_loop(0, n, body, 0)

    for src, dst_h in ((dk_s, dk_h), (dv_s, dv_h)):
      for_each(nb * npiece, lambda i, s=src, t=dst_h: win_out(s, t, i).start())
    zero_run(2 * nzero - issued[0])

    for c in grads_out:
      c.wait()
    for src, dst_h in ((dk_s, dk_h), (dv_s, dv_h)):
      for_each(nb * npiece, lambda i, s=src, t=dst_h: win_out(s, t, i).wait())
    for dst_h in (dk_h, dv_h):
      for_each(nzero, lambda i, t=dst_h: zero_out(t, i).wait())

  return kernel


@jax.jit
def pallas_interleave_layers__sliding_block_cached__dense_activation_gelu__decode_kernel(
    A_x: jax.Array,
    A_k_cache: jax.Array,
    A_v_cache: jax.Array,
    A_wq: jax.Array,
    A_wo: jax.Array,
    B_x: jax.Array,
    B_w1: jax.Array,
    B_b1: jax.Array,
    B_w2: jax.Array,
    B_b2: jax.Array,
    grad_out: jax.Array,
):
  del B_x
  nb, sq, d = A_x.shape
  _, hkv, seq, dh = A_k_cache.shape
  hd = A_wq.shape[1]
  rep = hd // (hkv * dh)
  f = B_w1.shape[1]
  win = min(4096, max(256, seq // 4))
  assert (nb, sq, rep, dh) == (2, 1, 4, 128)
  assert seq % _PIECE == 0 and win % 512 == 0

  zero_plan = (32, 8, 16, 8, 16, 8, 16, 16, 16, 8)
  kernel = _make_kernel(nb, hkv, rep, dh, seq, win, d, f, zero_plan)

  ins = (A_x.reshape(nb, d), grad_out.reshape(nb, d), A_k_cache, A_v_cache,
         A_wq, A_wo, B_w1, B_b1, B_w2, B_b2)
  out_shape = [jax.ShapeDtypeStruct(a.shape, a.dtype)
               for a in (ins[0], ins[0]) + ins[2:]]
  window = pltpu.VMEM((hkv, nb, win, dh), A_k_cache.dtype)

  def staged(arrs):
    return [window if a.ndim == 4 else pltpu.VMEM(a.shape, a.dtype)
            for a in arrs]

  hbm = pl.BlockSpec(memory_space=pltpu.HBM)
  res = pl.pallas_call(
      kernel,
      out_shape=out_shape,
      in_specs=[hbm] * len(ins),
      out_specs=[hbm] * len(out_shape),
      scratch_shapes=(
          staged(ins) + staged(out_shape)
          + [pltpu.VMEM((hkv, _PIECE, dh), A_k_cache.dtype)]
          + [pltpu.VMEM((hkv, 16, dh), _F32)] * 4
          + [pltpu.VMEM((hkv, 16, win), _F32)] * 2
          + [pltpu.SemaphoreType.DMA((8,)), pltpu.SemaphoreType.DMA((hkv,)),
             pltpu.SemaphoreType.DMA((hkv,)), pltpu.SemaphoreType.DMA((1,)),
             pltpu.SemaphoreType.DMA((1,))]),
      compiler_params=pltpu.CompilerParams(
          vmem_limit_bytes=120 * 1024 * 1024),
  )(*ins)
  return (res[0].reshape(A_x.shape), res[1].reshape(A_x.shape), *res[2:])
```

```python
import math

import jax
import jax.numpy as jnp
from jax import lax
import jax.experimental.pallas as pl
import jax.experimental.pallas.tpu as pltpu

_F32 = jnp.float32
_BF16 = jnp.bfloat16
_EPS = 1e-5
_GELU_C = math.sqrt(2.0 / math.pi)
_GELU_A = 0.044715

_PIECE = 112
_SLABS = (8, 8, 4, 4)
_ZERO_FIRST = 40
_ZERO_PER_HEAD = 8
_ZERO_BETWEEN = 16


def _mm(a, b):
  return lax.dot_general(a.astype(_BF16), b, (((1,), (0,)), ((), ())),
                         preferred_element_type=_F32)


def _mm_nt(a, b):
  return lax.dot_general(a.astype(_BF16), b, (((1,), (1,)), ((), ())),
                         preferred_element_type=_F32)


def _mm_tn(a, b):
  return lax.dot_general(a.astype(_BF16), b, (((0,), (0,)), ((), ())),
                         preferred_element_type=_F32)


def _rows(m, n):
  return lax.broadcasted_iota(jnp.int32, (m, n), 0)


def _ln_fwd(x):
  xc = x - jnp.mean(x, axis=-1, keepdims=True)
  var = jnp.mean(xc * xc, axis=-1, keepdims=True)
  rstd = 1.0 / jnp.sqrt(var + _EPS)
  return xc * rstd, rstd


def _ln_bwd(dn, n, rstd):
  return rstd * (dn - jnp.mean(dn, axis=-1, keepdims=True)
                 - n * jnp.mean(dn * n, axis=-1, keepdims=True))


def _gelu(h):
  t = jnp.tanh(_GELU_C * (h + _GELU_A * h * h * h))
  g = 0.5 * h * (1.0 + t)
  dg = 0.5 * (1.0 + t) + 0.5 * h * (1.0 - t * t) * _GELU_C * (
      1.0 + 3.0 * _GELU_A * h * h)
  return g, dg


def _sum_over_r(a):
  a = a + pltpu.roll(a, 4, 0)
  return a + pltpu.roll(a, 2, 0)


def _for(lo, hi, fn):
  def body(i, carry):
    fn(i)
    return carry

  lax.fori_loop(lo, hi, body, 0)


def _make_kernel(nb, hkv, rep, dh, seq, win, d, f):
  w0 = seq - win
  per_b = w0 // _PIECE
  nzero = nb * per_b
  scale = dh ** -0.5

  def kernel(x_h, go_h, k_h, v_h, wq_h, wo_h, w1_h, b1_h, w2_h, b2_h,
             out_h, dx_h, dk_h, dv_h, dwq_h, dwo_h, dw1_h, db1_h, dw2_h, db2_h,
             x_s, go_s, k_s, v_s, wq_s, wo_s, w1_s, b1_s, w2_s, b2_s,
             out_s, dx_s, dk_s, dv_s, dwq_s, dwo_s, dw1_s, db1_s, dw2_s, db2_s,
             z_s, q_s, o_s, do_s, dq_s, p_s, ds_s, sem):

    pairs = [(wq_h, wq_s), (x_h, x_s), (go_h, go_s), (b1_h, b1_s), (b2_h, b2_s)]
    for h in range(hkv):
      for src, dst in ((k_h, k_s), (v_h, v_s)):
        pairs.append((src.at[:, h, pl.ds(w0, win)], dst.at[:, h]))
    pairs += [(wo_h, wo_s), (w1_h, w1_s)]
    quarter = w2_s.shape[1] // 4
    for i in range(4):
      idx = (slice(None), pl.ds(i * quarter, quarter))
      pairs.append((w2_h.at[idx], w2_s.at[idx]))
    reads = [pltpu.make_async_copy(src, dst, sem.at[0])
             for src, dst in pairs[:-1]]
    last_read = pltpu.make_async_copy(*pairs[-1], sem.at[1])
    for c in reads + [last_read]:
      c.start()
    z_s[...] = jnp.zeros(z_s.shape, z_s.dtype)

    def zero_copy(which, i):
      row = pl.multiple_of((i % per_b) * _PIECE, 16)
      dst_h = (dk_h, dv_h)[which].at[i // per_b, :, pl.ds(row, _PIECE)]
      return pltpu.make_async_copy(z_s, dst_h, sem.at[0])

    queued = [0]

    def zero_run(n):
      while n > 0:
        which, lo = divmod(queued[0], nzero)
        m = min(n, nzero - lo)
        _for(lo, lo + m, lambda i, which=which: zero_copy(which, i).start())
        queued[0] += m
        n -= m

    def head_loop(fn):
      which, lo = divmod(queued[0], nzero)
      assert lo + _ZERO_PER_HEAD * hkv <= nzero
      queued[0] += _ZERO_PER_HEAD * hkv

      def step(h):
        _for(0, _ZERO_PER_HEAD,
             lambda i: zero_copy(which, lo + h * _ZERO_PER_HEAD + i).start())
        fn(h)

      _for(0, hkv, step)

    odd_d = _rows(8, d) % 2 == 1
    odd_h = _rows(8, dh) % 2 == 1
    odd_w = _rows(8, win) % 2 == 1
    r_h = _rows(8, dh) // 2

    def weight(ref):
      return ref[...].reshape(-1, ref.shape[-1])

    def load_pair(ref):
      return jnp.where(odd_d,
                       jnp.broadcast_to(ref[1:2].astype(_F32), (8, d)),
                       jnp.broadcast_to(ref[0:1].astype(_F32), (8, d)))

    def to_heads(big, dst, layer):
      for h in range(hkv):
        t = big[:, h * rep * dh:(h * rep + 1) * dh]
        for r in range(1, rep):
          j = h * rep + r
          t = jnp.where(r_h == r, big[:, j * dh:(j + 1) * dh], t)
        dst[h, layer * 8:(layer + 1) * 8, :] = t

    def from_heads(src, layer):
      tiles = []
      for h in range(hkv):
        t = src[h, layer * 8:(layer + 1) * 8, :]
        for r in range(rep):
          tiles.append(jnp.where(r_h == r, t, 0.0))
      return jnp.concatenate(tiles, axis=1)

    def attn_fwd(x, layer):
      n, rstd = _ln_fwd(x)
      to_heads(_mm(n, weight(wq_s)), q_s, layer)
      rows = slice(layer * 8, (layer + 1) * 8)

      def head(h):
        q = q_s[h, rows, :]
        s = jnp.where(odd_w, _mm_nt(q, k_s[1, h]), _mm_nt(q, k_s[0, h])) * scale
        e = jnp.exp(s - jnp.max(s, axis=-1, keepdims=True))
        p = e / jnp.sum(e, axis=-1, keepdims=True)
        p_s[h, rows, :] = p
        o_s[h, rows, :] = jnp.where(odd_h, _mm(p, v_s[1, h]), _mm(p, v_s[0, h]))

      head_loop(head)
      y = x + _sum_over_r(_mm(from_heads(o_s, layer), weight(wo_s)))
      return y, n, rstd

    def attn_bwd(dy, layer, n, rstd):
      to_heads(_mm_nt(dy, weight(wo_s)), do_s, layer)
      rows = slice(layer * 8, (layer + 1) * 8)

      def head(h):
        do = do_s[h, rows, :]
        p = p_s[h, rows, :]
        dp = jnp.where(odd_w, _mm_nt(do, v_s[1, h]), _mm_nt(do, v_s[0, h]))
        ds = p * (dp - jnp.sum(p * dp, axis=-1, keepdims=True)) * scale
        ds_s[h, rows, :] = ds
        dq_s[h, rows, :] = jnp.where(
            odd_h, _mm(ds, k_s[1, h]), _mm(ds, k_s[0, h]))

      head_loop(head)
      dn = _sum_over_r(_mm_nt(from_heads(dq_s, layer), weight(wq_s)))
      return dy + _ln_bwd(dn, n, rstd)

    def mlp_fwd(x, b1, b2):
      n, rstd = _ln_fwd(x)
      g, dg = _gelu(_mm(n, weight(w1_s)) + b1)
      return x + _mm(g, weight(w2_s)) + b2, n, rstd, g, dg

    def mlp_bwd(dy, n, rstd, dg):
      dpre = _mm_nt(dy, weight(w2_s)) * dg
      return dy + _ln_bwd(_mm_nt(dpre, weight(w1_s)), n, rstd), dpre

    for c in reads:
      c.wait()
    zero_run(_ZERO_FIRST)
    last_read.wait()

    x0 = load_pair(x_s)
    b1 = b1_s[...].astype(_F32).reshape(1, f)
    b2 = b2_s[...].astype(_F32).reshape(1, d)
    x1, n1, rstd1 = attn_fwd(x0, 0)
    zero_run(_ZERO_BETWEEN)
    x2, n2, rstd2, act2, dact2 = mlp_fwd(x1, b1, b2)
    x3, n3, rstd3 = attn_fwd(x2, 1)
    zero_run(_ZERO_BETWEEN)
    x4, n4, rstd4, act4, dact4 = mlp_fwd(x3, b1, b2)
    out_s[...] = x4[0:nb].astype(out_s.dtype)

    g4 = load_pair(go_s)
    g3, dpre4 = mlp_bwd(g4, n4, rstd4, dact4)
    g2 = attn_bwd(g3, 1, n3, rstd3)
    zero_run(_ZERO_BETWEEN)
    g1, dpre2 = mlp_bwd(g2, n2, rstd2, dact2)
    g0 = attn_bwd(g1, 0, n1, rstd1)
    dx_s[...] = g0[0:nb].astype(dx_s.dtype)

    def both(a, b):
      return jnp.concatenate([a, b], axis=0)

    def one_r(a):
      return jnp.where(_rows(*a.shape) < nb, a, 0.0)

    def outer(a, b, dst, chunk):
      b = b.astype(_BF16)
      slab = dst.shape[1]
      for i in range(0, a.shape[1], chunk):
        r = _mm_tn(a[:, i:i + chunk], b).astype(dst.dtype)
        j = i
        while j < i + chunk:
          m = min(i + chunk - j, slab - j % slab)
          dst[j // slab, j % slab:j % slab + m, :] = r[j - i:j - i + m]
          j += m

    zero_run(_ZERO_BETWEEN)
    dym = both(one_r(g2), one_r(g4))
    dpre = both(one_r(dpre2), one_r(dpre4))
    db2_s[...] = jnp.sum(dym, axis=0, keepdims=True).reshape(d).astype(db2_s.dtype)
    db1_s[...] = jnp.sum(dpre, axis=0, keepdims=True).reshape(f).astype(db1_s.dtype)
    outer(both(n2, n4), dpre, dw1_s, 128)
    outer(both(act2, act4), dym, dw2_s, 256)
    zero_run(_ZERO_BETWEEN)
    outer(both(n1, n3), both(from_heads(dq_s, 0), from_heads(dq_s, 1)),
          dwq_s, 128)
    zero_run(_ZERO_BETWEEN)
    outer(both(from_heads(o_s, 0), from_heads(o_s, 1)), both(g1, g3),
          dwo_s, 512)

    writes = [pltpu.make_async_copy(src, dst, sem.at[0]) for src, dst in (
        (out_s, out_h), (dx_s, dx_h), (db1_s, db1_h), (db2_s, db2_h))]

    def add_slabs(src, dst_h, row, rows, col=0, cols=None):
      cols = src.shape[2] if cols is None else cols
      idx = (slice(None), pl.ds(row, rows), pl.ds(col, cols))
      writes.append(
          pltpu.make_async_copy(src.at[idx], dst_h.at[idx], sem.at[0]))

    half = dwq_s.shape[2] // 2
    for row in range(0, dwq_s.shape[1], 8):
      for col in (0, half):
        add_slabs(dwq_s, dwq_h, row, 8, col, half)
    for row in range(0, dwo_s.shape[1], 32):
      add_slabs(dwo_s, dwo_h, row, 32)
    for i in range(max(dw1_s.shape[1] // 8, dw2_s.shape[1] // 32)):
      if i * 8 < dw1_s.shape[1]:
        add_slabs(dw1_s, dw1_h, i * 8, 8)
      if i * 32 < dw2_s.shape[1]:
        add_slabs(dw2_s, dw2_h, i * 32, 32)
    for c in writes:
      c.start()

    odd_2h = _rows(16, dh) % 2 == 1

    def cache_grads(h):
      for lhs_s, rhs_s, dst in ((ds_s, q_s, dk_s), (p_s, do_s, dv_s)):
        t = rhs_s[h]
        rhs = jnp.concatenate(
            [jnp.where(odd_2h, 0.0, t), jnp.where(odd_2h, t, 0.0)],
            axis=1).astype(_BF16)
        for i in range(0, win, 512):
          r = _mm_tn(lhs_s[h, :, i:i + 512], rhs).astype(dst.dtype)
          dst[0, h, i:i + 512, :] = r[:, :dh]
          dst[1, h, i:i + 512, :] = r[:, dh:]

    head_loop(cache_grads)

    def window_copies(act):
      npiece, rest = divmod(win, _PIECE)
      for src, dst_h in ((dk_s, dk_h), (dv_s, dv_h)):
        for b in range(nb):
          def copy(row, rows, src=src, dst_h=dst_h, b=b):
            return pltpu.make_async_copy(
                src.at[b, :, pl.ds(row, rows)],
                dst_h.at[b, :, pl.ds(w0 + row, rows)], sem.at[0])

          _for(0, npiece, lambda i, copy=copy: act(
              copy(pl.multiple_of(i * _PIECE, 16), _PIECE)))
          if rest:
            act(copy(npiece * _PIECE, rest))

    window_copies(lambda c: c.start())
    zero_run(2 * nzero - queued[0])

    for c in writes:
      c.wait()
    window_copies(lambda c: c.wait())
    for which in range(2):
      _for(0, nzero, lambda i, which=which: zero_copy(which, i).wait())

  return kernel


@jax.jit
def pallas_interleave_layers__sliding_block_cached__dense_activation_gelu__decode_kernel(
    A_x: jax.Array,
    A_k_cache: jax.Array,
    A_v_cache: jax.Array,
    A_wq: jax.Array,
    A_wo: jax.Array,
    B_x: jax.Array,
    B_w1: jax.Array,
    B_b1: jax.Array,
    B_w2: jax.Array,
    B_b2: jax.Array,
    grad_out: jax.Array,
):
  del B_x
  nb, sq, d = A_x.shape
  _, hkv, seq, dh = A_k_cache.shape
  rep = A_wq.shape[1] // (hkv * dh)
  f = B_w1.shape[1]
  win = min(4096, max(256, seq // 4))
  assert (nb, sq, rep, dh) == (2, 1, 4, 128)
  assert (seq - win) % _PIECE == 0 and win % 512 == 0

  kernel = _make_kernel(nb, hkv, rep, dh, seq, win, d, f)

  wq, wo, w1, w2 = (w.reshape(n, w.shape[0] // n, w.shape[1])
                    for w, n in zip((A_wq, A_wo, B_w1, B_w2), _SLABS))
  ins = (A_x.reshape(nb, d), grad_out.reshape(nb, d), A_k_cache, A_v_cache,
         wq, wo, w1, B_b1, w2, B_b2)
  out_shape = [jax.ShapeDtypeStruct(a.shape, a.dtype)
               for a in (ins[0], ins[0]) + ins[2:]]

  def staged(arrs):
    return [pltpu.VMEM((nb, hkv, win, dh) if a.ndim == 4 else a.shape, a.dtype)
            for a in arrs]

  hbm = pl.BlockSpec(memory_space=pltpu.HBM)
  res = pl.pallas_call(
      kernel,
      out_shape=out_shape,
      in_specs=[hbm] * len(ins),
      out_specs=[hbm] * len(out_shape),
      scratch_shapes=(
          staged(ins) + staged(out_shape)
          + [pltpu.VMEM((hkv, _PIECE, dh), A_k_cache.dtype)]
          + [pltpu.VMEM((hkv, 16, dh), _F32)] * 4
          + [pltpu.VMEM((hkv, 16, win), _F32)] * 2
          + [pltpu.SemaphoreType.DMA((2,))]),
      compiler_params=pltpu.CompilerParams(
          vmem_limit_bytes=112 * 1024 * 1024),
  )(*ins)
  like = (A_x, A_x, A_k_cache, A_v_cache, A_wq, A_wo, B_w1, B_b1, B_w2, B_b2)
  return tuple(r.reshape(a.shape) for r, a in zip(res, like))
```
